```python
import os as _os
_os.environ.setdefault("JAX_PLATFORMS", "cpu")
import jax
import jax.numpy as jnp

def _softmax(x, axis=-1):
    return jax.nn.softmax(x, axis=axis)
def _gelu(x):
    return jax.nn.gelu(x, approximate=True)
def _silu(x):
    return jax.nn.silu(x)
def _sigmoid(x):
    return jax.nn.sigmoid(x)
def _layernorm(x, axis=-1, eps=1e-5):
    m = jnp.mean(x, axis=axis, keepdims=True)
    v = jnp.var(x, axis=axis, keepdims=True)
    return (x - m) / jnp.sqrt(v + eps)
def _scatter_add(tgt, idx, src, axis=0):
    return tgt.at[idx].add(src)
def _segment_sum(src, seg, n):
    return jax.ops.segment_sum(src, seg, n)
class _Rng:
    def __init__(self, key):
        self._k = key
    def _next(self):
        self._k, sub = jax.random.split(self._k)
        return sub
    def normal(self, shape):
        return jax.random.normal(self._next(), shape, dtype=jnp.bfloat16)
    def randint(self, lo, hi, shape):
        return jax.random.randint(self._next(), shape, lo, hi, dtype=jnp.int32)
    def uniform(self, shape, lo=0.0, hi=1.0):
        return jax.random.uniform(self._next(), shape, jnp.bfloat16, lo, hi)
    def permutation(self, n):
        return jax.random.permutation(self._next(), n)


kernel_name = 'gated_mix__sliding_block__dense_activation_silu__prompt'

def setup_inputs():
    _rng = _Rng(jax.random.key(int.from_bytes(__import__("os").urandom(4), "little")))
    _w = (lambda a: (lambda t: t.astype(jnp.bfloat16) if jnp.issubdtype(t.dtype, jnp.floating) else t)(jnp.asarray(a)))
    def _A_setup():
        B, S, D = 1, 2048, 640
        return {
            "x": _w((lambda *s: _rng.normal(s) * 0.05)(B, S, D)),
            "wqkv": _w((lambda *s: _rng.normal(s) * 0.4)(D, 3 * D)),
            "wo": _w((lambda *s: _rng.normal(s) * 0.05)(D, D)),
        }
    _A_in = _A_setup()

    def _B_setup():
        B, S, D, F = 1, 2048, 640, 1536
        return {
            "x": _w((lambda *s: _rng.normal(s) * 0.05)(B, S, D)),
            "w1": _w((lambda *s: _rng.normal(s) * 1.6)(D, F) * (D ** -0.5)),
            "w2": _w((lambda *s: _rng.normal(s) * 1.6)(F, D) * (F ** -0.5)),
        }
    _B_in = _B_setup()

    return {
        "A_x": _A_in["x"],
        "A_wqkv": _A_in["wqkv"],
        "A_wo": _A_in["wo"],
        "B_x": _B_in["x"],
        "B_w1": _B_in["w1"],
        "B_w2": _B_in["w2"],
        "gate_w": _w((lambda *s: _rng.normal(s) * 0.05)(640) * 16.0),
    }

def reference(A_x, A_wqkv, A_wo, B_x, B_w1, B_w2, gate_w):
    def _A_ref(x, wqkv, wo):
        B, S, D = x.shape
        H = 32; Dh = D // H; W = 256
        qkv = (lambda x, *d: x.transpose(*d))((x @ wqkv).reshape(B, S, 3, H, Dh), 2, 0, 3, 1, 4)
        q, k, v = qkv[0], qkv[1], qkv[2]
        scores = jnp.einsum("bhqd,bhkd->bhqk", q, k) * (Dh ** -0.5)
        idx = jnp.arange(S)
        mask = (idx[:, None] - idx[None, :] >= 0) & (idx[:, None] - idx[None, :] < W)
        scores = jnp.where(mask[None, None], scores, -1e9)
        p = _softmax(scores, axis=-1)
        o = jnp.einsum("bhqk,bhkd->bhqd", p, v)
        return (lambda x, *d: x.transpose(*d))(o, 0, 2, 1, 3).reshape(B, S, D) @ wo

    def _B_ref(x, w1, w2):
        h = jnp.einsum("bsd,df->bsf", x, w1)
        h = _silu(h)
        out = jnp.einsum("bsf,fd->bsd", h, w2)
        return out

    x = A_x
    g = _sigmoid((x * gate_w).sum(-1, keepdims=True))
    a = _A_ref(x, A_wqkv, A_wo)
    b = _B_ref(x, B_w1, B_w2)
    return g * a + (1 - g) * b
```

```python
import functools
import numpy as np
import jax
import jax.numpy as jnp
from jax import lax
import jax.experimental.pallas as pl
import jax.experimental.pallas.tpu as pltpu

S = 2048
D = 640
F = 1536
H = 32
DH = 20
W = 256
BQ = 256
NG = 8
NEG = -1e30
LOG2E = float(np.log2(np.e))
QSCALE = LOG2E * (DH ** -0.5)
NT = (((1,), (1,)), ((), ()))
SLAB_START = [0, 64, 128, 192, 320, 384, 448, 512]
DEN_LO = 2.0 ** -60


def _lane_of(g, col):
    st = SLAB_START[g]
    if st % 128 == 0:
        return col - st
    return (col - st + 64) % 128


def _head_lane0(h):
    return _lane_of(h // 4, DH * h)


def _slab(v, g, lane_hi):
    st = SLAB_START[g]
    if st % 128 == 0:
        return v[:, st:st + 128]
    m = st // 128
    return jnp.where(lane_hi, v[:, 128 * m:128 * (m + 1)], v[:, 128 * (m + 1):128 * (m + 2)])


def _win(h):
    w0 = 16 * ((DH * h) // 16)
    o = DH * h - w0
    r = 31 if o <= 8 else 0
    return w0, o, r


def _pack(x):
    return pltpu.bitcast(x.astype(jnp.bfloat16), jnp.uint32)


def _unpack(x):
    return pltpu.bitcast(x, jnp.bfloat16)


def _kernel(x_hbm, wqkv_hbm, wo_hbm, w1_hbm, w2_hbm, gw_hbm, o_ref,
            x_buf, wqkv_ref, wo_ref, w1_ref, w2_ref, gw_ref,
            k_scr, vt_scr, qm_scr, p0, p1, ot_scr, h_scr, b_scr, g_scr, bias_scr,
            xsem, wsem):
    i = pl.program_id(0)
    n_steps = S // BQ
    zero = jnp.minimum(i, 0)
    z16 = pl.multiple_of(zero * 16, 16)
    slot = i % 2

    def x_copy(blk, sl):
        return pltpu.make_async_copy(x_hbm.at[pl.ds(pl.multiple_of(blk * BQ, BQ), BQ), :], x_buf.at[sl], xsem.at[sl])

    cp_k = pltpu.make_async_copy(wqkv_hbm.at[:, pl.ds(D, D)], wqkv_ref.at[:, pl.ds(D, D)], wsem.at[0])
    cp_q = pltpu.make_async_copy(wqkv_hbm.at[:, pl.ds(0, D)], wqkv_ref.at[:, pl.ds(0, D)], wsem.at[1])
    cp_v = pltpu.make_async_copy(wqkv_hbm.at[:, pl.ds(2 * D, D)], wqkv_ref.at[:, pl.ds(2 * D, D)], wsem.at[2])
    cp_1 = pltpu.make_async_copy(w1_hbm, w1_ref, wsem.at[3])
    cp_2 = pltpu.make_async_copy(w2_hbm, w2_ref, wsem.at[4])
    cp_o = pltpu.make_async_copy(wo_hbm, wo_ref, wsem.at[5])
    cp_g = pltpu.make_async_copy(gw_hbm, gw_ref, wsem.at[6])

    def body(first):
        if first:
            x_copy(0, 0).start()
            cp_k.start()
            cp_q.start(priority=1)
            cp_v.start(priority=1)
            cp_g.start(priority=1)
            cp_1.start(priority=1)
            cp_2.start(priority=1)
            cp_o.start(priority=1)
            x_copy(1, 1).start(priority=1)
            ri = lax.broadcasted_iota(jnp.int32, (128, 128), 0)
            li = lax.broadcasted_iota(jnp.int32, (128, 128), 1)
            bias_scr[pl.ds(0, 128), :] = jnp.where(ri > li, 0.0, NEG)
            bias_scr[pl.ds(128, 128), :] = jnp.where(ri <= li, 0.0, NEG)
            x_copy(0, 0).wait()
            x = x_buf[0]
            cp_k.wait()
        else:
            x_copy(i, slot).wait()
            x = x_buf[slot]

        lane_hi = lax.broadcasted_iota(jnp.int32, (BQ, 128), 1) >= 64

        k = jnp.dot(x, wqkv_ref[:, D:2 * D], preferred_element_type=jnp.float32)
        kext = jnp.concatenate([_slab(k, g, lane_hi) for g in range(NG)], axis=1)
        if first:
            k_scr[pl.ds(0, BQ // 2), :] = _pack(kext)
            cp_q.wait()
        else:
            k_scr[pl.ds(pl.multiple_of(i * (BQ // 2), 128), BQ // 2), :] = _pack(kext)

        q = jnp.dot(x, wqkv_ref[:, 0:D], preferred_element_type=jnp.float32)
        lane1 = lax.broadcasted_iota(jnp.int32, (1, 128), 1)
        for g in range(NG):
            qg = _slab(q, g, lane_hi)
            for hh in range(4):
                h = 4 * g + hh
                lm = jnp.where(((lane1 - _head_lane0(h)) & 127) < DH, QSCALE, 0.0)
                qm = _pack(qg * lm)
                qm_scr[h, 0] = qm[0:64]
                qm_scr[h, 1] = qm[64:128]
        if first:
            cp_v.wait()
            cp_g.wait()

        v = jnp.dot(x, wqkv_ref[:, 2 * D:3 * D], preferred_element_type=jnp.float32)
        vt = v.T
        row32 = lax.broadcasted_iota(jnp.int32, (32, BQ), 0)
        for h in range(H):
            w0, o, r = _win(h)
            win = jnp.where(row32 == r, 1.0, vt[w0:w0 + 32, :])
            if first:
                vt_scr[h, :, pl.ds(0, BQ)] = _pack(win)
            else:
                vt_scr[h, :, pl.ds(pl.multiple_of(i * BQ, 256), BQ)] = _pack(win)

        gl = jnp.sum(x.astype(jnp.float32) * gw_ref[...].astype(jnp.float32).reshape(1, D), axis=-1, keepdims=True)
        g_scr[...] = jnp.broadcast_to(0.5 * jnp.tanh(0.5 * gl) + 0.5, (BQ, 128))

        def ffn1():
            hpre = jnp.dot(x, w1_ref[...], preferred_element_type=jnp.float32)
            u = 0.5 * hpre
            h_scr[...] = _pack(u * jnp.tanh(u) + u)

        def ffn2(c0=0, c1=D):
            b_scr[:, c0:c1] = jnp.dot(_unpack(h_scr[...]), w2_ref[:, c0:c1], preferred_element_type=jnp.float32)

        units = [(j, g) for j in range(BQ // 128) for g in range(NG)]
        pb = [p0, p1]
        outs = [None] * H
        dmin = [None]
        dmax = [None]
        row8 = lax.broadcasted_iota(jnp.int32, (8, 128), 0)

        def nkeys(j):
            return 384 if not first else 128 * (j + 1)

        def stage_qk(t):
            j, g = units[t]
            nk = nkeys(j)
            if first:
                kw = _unpack(k_scr[pl.ds(0, nk // 2), pl.ds(g * 128, 128)])
            else:
                kw = _unpack(k_scr[pl.ds(pl.multiple_of(i * 128 + j * 64 - 128, 64), 192), pl.ds(g * 128, 128)])
            qst = _unpack(qm_scr[pl.ds(4 * g, 4), j].reshape(256, 128))
            s4 = lax.dot_general(kw, qst, NT, preferred_element_type=jnp.float32)
            parts = []
            if nk == 384:
                bA = bias_scr[pl.ds(0, 128), :]
                parts.append(s4[0:128] + jnp.concatenate([bA] * 4, axis=1))
            if nk >= 256:
                parts.append(s4[nk - 256:nk - 128])
            bC = bias_scr[pl.ds(128, 128), :]
            parts.append(s4[nk - 128:nk] + jnp.concatenate([bC] * 4, axis=1))
            p = jnp.exp2(jnp.concatenate(parts, axis=0))
            pb[t % 2][pl.ds(z16, nk // 2), :] = _pack(p)

        def stage_pv(t):
            j, g = units[t]
            nk = nkeys(j)
            for hh in range(4):
                h = 4 * g + hh
                p = _unpack(pb[t % 2][pl.ds(z16, nk // 2), pl.ds(hh * 128, 128)])
                if first:
                    vw = _unpack(vt_scr[h, :, pl.ds(0, nk)])
                else:
                    vw = _unpack(vt_scr[h, :, pl.ds(pl.multiple_of(i * BQ + j * 128 - 256, 128), 384)])
                out = jnp.dot(vw, p, preferred_element_type=jnp.float32)
                w0, o, r = _win(h)
                den = out[r:r + 1, :]
                dmin[0] = den if dmin[0] is None else jnp.minimum(dmin[0], den)
                dmax[0] = den if dmax[0] is None else jnp.maximum(dmax[0], den)
                outs[h] = out * (1.0 / den)
                if hh % 2 == 1:
                    R0 = (DH * (h - 1)) // 8
                    pieces = []
                    for R in range(R0, R0 + 5):
                        h1 = (8 * R) // DH
                        h2 = (8 * R + 7) // DH
                        w1_, _, _ = _win(h1)
                        p1_ = outs[h1][8 * R - w1_:8 * R - w1_ + 8]
                        if h2 != h1:
                            w2_, _, _ = _win(h2)
                            p2_ = outs[h2][8 * R - w2_:8 * R - w2_ + 8]
                            p1_ = jnp.where(row8 < DH * h2 - 8 * R, p1_, p2_)
                        pieces.append(p1_)
                    ot_scr[pl.ds(8 * R0, 40), pl.ds(j * 128, 128)] = jnp.concatenate(pieces, axis=0)

        def attention(filler=None):
            n = len(units)
            stage_qk(0)
            for t in range(n):
                if t + 1 < n:
                    stage_qk(t + 1)
                elif filler is not None:
                    filler()
                stage_pv(t)

        if first:
            attention()
            cp_1.wait()
            ffn1()
            cp_2.wait()
            ffn2()
            cp_o.wait()
        else:
            ffn1()
            attention(lambda: ffn2(0, 256))
            ffn2(256, D)

        def finalize():
            o = ot_scr[...].T.astype(jnp.bfloat16)
            a = jnp.dot(o, wo_ref[...], preferred_element_type=jnp.float32)
            b = b_scr[...]
            g = jnp.concatenate([g_scr[...]] * (D // 128), axis=1)
            o_ref[...] = (b + g * (a - b)).astype(o_ref.dtype)

        omax = jnp.max(jnp.abs(ot_scr[...]), axis=0, keepdims=True)
        ok = jnp.logical_and(dmin[0] >= DEN_LO, dmax[0] < jnp.inf)
        ok = jnp.logical_and(ok, jnp.logical_and(omax[:, 0:128] < jnp.inf, omax[:, 128:256] < jnp.inf))
        nbad = jnp.max(jnp.where(ok, 0, 1))
        finalize()

        @pl.when(nbad > 0)
        def _():
            nk = 256 if first else 384
            ri = lax.broadcasted_iota(jnp.int32, (nk, 128), 0)
            li = lax.broadcasted_iota(jnp.int32, (nk, 128), 1)
            row = lax.broadcasted_iota(jnp.int32, (32, 128), 0)

            def loop(t, carry):
                j = t // H
                h = t % H
                g = h // 4
                q0 = i * BQ + j * 128
                k0 = 0 if first else q0 - 256
                kw = _unpack(k_scr[pl.ds(pl.multiple_of(k0 // 2, 64), nk // 2), pl.ds(pl.multiple_of(g * 128, 128), 128)])
                s = lax.dot_general(kw, _unpack(qm_scr[h, j]), NT, preferred_element_type=jnp.float32)
                dist = (q0 + li) - (k0 + ri)
                s = jnp.where((dist >= 0) & (dist < W), s, NEG)
                m = jnp.max(s, axis=0, keepdims=True)
                p = jnp.exp2(s - m).astype(jnp.bfloat16)
                vw = _unpack(vt_scr[h, :, pl.ds(pl.multiple_of(k0, 128), nk)])
                out = jnp.dot(vw, p, preferred_element_type=jnp.float32)
                w0 = ((DH * h) // 16) * 16
                o = DH * h - w0
                r = jnp.where(o <= 8, 31, 0)
                den = jnp.sum(jnp.where(row == r, out, 0.0), axis=0, keepdims=True)
                sl = (pl.ds(pl.multiple_of(w0, 16), 32), pl.ds(pl.multiple_of(j * 128, 128), 128))
                old = ot_scr[sl]
                ot_scr[sl] = jnp.where((row >= o) & (row < o + DH), out * (1.0 / den), old)
                return carry

            lax.fori_loop(0, 2 * H, loop, 0)
            finalize()

    @pl.when(i == 0)
    def _():
        body(True)

    @pl.when(i > 0)
    def _():
        @pl.when(i + 1 < n_steps)
        def _():
            x_copy(i + 1, 1 - slot).start()
        body(False)


@jax.jit
def pallas_gated_mix__sliding_block__dense_activation_silu__prompt_kernel(
    A_x: jax.Array,
    A_wqkv: jax.Array,
    A_wo: jax.Array,
    B_x: jax.Array,
    B_w1: jax.Array,
    B_w2: jax.Array,
    gate_w: jax.Array,
):
    del B_x
    x2 = A_x.reshape(S, D)
    anyspec = pl.BlockSpec(memory_space=pl.ANY)
    const = lambda i: (0, 0)
    out = pl.pallas_call(
        _kernel,
        grid=(S // BQ,),
        in_specs=[
            anyspec, anyspec, anyspec, anyspec, anyspec,
            anyspec,
        ],
        out_specs=pl.BlockSpec((BQ, D), lambda i: (i, 0)),
        out_shape=jax.ShapeDtypeStruct((S, D), A_x.dtype),
        scratch_shapes=[
            pltpu.VMEM((2, BQ, D), jnp.bfloat16),
            pltpu.VMEM((D, 3 * D), jnp.bfloat16),
            pltpu.VMEM((D, D), jnp.bfloat16),
            pltpu.VMEM((D, F), jnp.bfloat16),
            pltpu.VMEM((F, D), jnp.bfloat16),
            pltpu.VMEM((D,), jnp.bfloat16),
            pltpu.VMEM((S // 2, NG * 128), jnp.uint32),
            pltpu.VMEM((H, 16, S), jnp.uint32),
            pltpu.VMEM((H, 2, 64, 128), jnp.uint32),
            pltpu.VMEM((192 + 16, 512), jnp.uint32),
            pltpu.VMEM((192 + 16, 512), jnp.uint32),
            pltpu.VMEM((D, BQ), jnp.float32),
            pltpu.VMEM((BQ // 2, F), jnp.uint32),
            pltpu.VMEM((BQ, D), jnp.float32),
            pltpu.VMEM((BQ, 128), jnp.float32),
            pltpu.VMEM((256, 128), jnp.float32),
            pltpu.SemaphoreType.DMA((2,)),
            pltpu.SemaphoreType.DMA((7,)),
        ],
        compiler_params=pltpu.CompilerParams(
            dimension_semantics=("arbitrary",),
            vmem_limit_bytes=100 * 1024 * 1024,
        ),
    )(x2, A_wqkv, A_wo, B_w1, B_w2, gate_w)
    return out.reshape(1, S, D)
```

```python
import numpy as np
import jax
import jax.numpy as jnp
from jax import lax
import jax.experimental.pallas as pl
import jax.experimental.pallas.tpu as pltpu

S = 2048
D = 640
F = 1536
H = 32
DH = 20
W = 256
BQ = 256
NJ = BQ // 128
NG = 8
VR = 24
NEG = -1e30
QSCALE = float(np.log2(np.e)) * (DH ** -0.5)
SLAB_START = (0, 64, 128, 192, 320, 384, 448, 512)
DEN_LO = 2.0 ** -60
KC = 256


def _head_lane0(h):
    st = SLAB_START[h // 4]
    col = DH * h
    return col - st if st % 128 == 0 else (col - st + 64) % 128


def _slab(v, g, lane_hi):
    st = SLAB_START[g]
    if st % 128 == 0:
        return v[:, st:st + 128]
    m = st // 128
    return jnp.where(lane_hi, v[:, 128 * m:128 * (m + 1)], v[:, 128 * (m + 1):128 * (m + 2)])


def _pack(x):
    return pltpu.bitcast(x.astype(jnp.bfloat16), jnp.uint32)


def _unpack(x):
    return pltpu.bitcast(x, jnp.bfloat16)


def _al(x, n):
    return x if isinstance(x, int) else pl.multiple_of(x, n)


def _kernel(x_hbm, wqkv_hbm, wo_hbm, w1_hbm, w2_hbm, gw_hbm, o_ref,
            x_buf, wqkv_ref, wo_ref, w1_ref, w2_ref, gw_ref,
            k_scr, vt_scr, qm_scr, p0, p1, ot_scr, h_scr, b_scr, g_scr, bias_scr,
            xsem, wsem):
    i = pl.program_id(0)
    n_steps = S // BQ
    z16 = pl.multiple_of(jnp.minimum(i, 0) * 16, 16)
    slot = i % 2

    def x_copy(blk, sl):
        return pltpu.make_async_copy(x_hbm.at[pl.ds(_al(blk * BQ, BQ), BQ), :], x_buf.at[sl], xsem.at[sl])

    def w_copy(src, dst, sem):
        return pltpu.make_async_copy(src, dst, wsem.at[sem])

    cp_k0 = w_copy(wqkv_hbm.at[:, pl.ds(D, KC)], wqkv_ref.at[:, pl.ds(D, KC)], 0)
    cp_k1 = w_copy(wqkv_hbm.at[:, pl.ds(D + KC, D - KC)], wqkv_ref.at[:, pl.ds(D + KC, D - KC)], 1)
    cp_q = w_copy(wqkv_hbm.at[:, pl.ds(0, D)], wqkv_ref.at[:, pl.ds(0, D)], 2)
    cp_v = w_copy(wqkv_hbm.at[:, pl.ds(2 * D, D)], wqkv_ref.at[:, pl.ds(2 * D, D)], 3)
    cp_g = w_copy(gw_hbm, gw_ref, 4)
    cp_1 = w_copy(w1_hbm, w1_ref, 5)
    cp_2 = w_copy(w2_hbm, w2_ref, 6)
    cp_o = w_copy(wo_hbm, wo_ref, 7)

    def body(first):
        blk = 0 if first else i
        if first:
            x_copy(0, 0).start()
            cp_k0.start()
            for cp in (cp_k1, cp_q, cp_v, cp_g, cp_1, cp_2, cp_o, x_copy(1, 1)):
                cp.start(priority=1)
            ri = lax.broadcasted_iota(jnp.int32, (32, 128), 0)
            li = lax.broadcasted_iota(jnp.int32, (32, 128), 1) % 32
            bias_scr[pl.ds(0, 32), :] = jnp.where(ri > li, 0.0, NEG)
            bias_scr[pl.ds(32, 32), :] = jnp.where(ri <= li, 0.0, NEG)
            x_copy(0, 0).wait()
            cp_k0.wait()
            x = x_buf[0]
        else:
            x_copy(i, slot).wait()
            x = x_buf[slot]

        lane_hi = lax.broadcasted_iota(jnp.int32, (BQ, 128), 1) >= 64
        lane1 = lax.broadcasted_iota(jnp.int32, (1, 128), 1)

        def proj(c0, c1):
            return jnp.dot(x, wqkv_ref[:, c0:c1], preferred_element_type=jnp.float32)

        def post_k(k):
            kext = jnp.concatenate([_slab(k, g, lane_hi) for g in range(NG)], axis=1)
            k_scr[pl.ds(_al(blk * (BQ // 2), BQ // 2), BQ // 2), :] = _pack(kext)

        def post_q(q):
            for g in range(NG):
                qg = _slab(q, g, lane_hi)
                lms = [jnp.where(((lane1 - _head_lane0(4 * g + hh)) & 127) < DH, QSCALE, 0.0)
                       for hh in range(4)]
                for j in range(NJ):
                    for t in range(4):
                        rows = qg[128 * j + 32 * t:128 * j + 32 * t + 32]
                        tile = jnp.concatenate(
                            [(rows * lms[c ^ t]).astype(jnp.bfloat16) for c in range(4)], axis=0)
                        qm_scr[j, g, t] = pltpu.bitcast(tile.T, jnp.uint32)

        def post_v(v):
            vt = v.T.astype(jnp.bfloat16).astype(jnp.float32)
            rowv = lax.broadcasted_iota(jnp.int32, (VR, BQ), 0)
            for h in range(H):
                w0 = 8 * ((DH * h) // 8)
                ones_row = VR - 1 if h % 2 == 0 else 0
                vt_scr[h, :, pl.ds(_al(blk * BQ, BQ), BQ)] = jnp.where(
                    rowv == ones_row, 1.0, vt[w0:w0 + VR, :])

        def gate():
            gw = gw_ref[...].astype(jnp.float32).reshape(1, D)
            gl = jnp.sum(x.astype(jnp.float32) * gw, axis=-1, keepdims=True)
            g_scr[...] = jnp.broadcast_to(0.5 * jnp.tanh(0.5 * gl) + 0.5, (BQ, 128))

        def ffn1():
            u = 0.5 * jnp.dot(x, w1_ref[...], preferred_element_type=jnp.float32)
            h_scr[...] = _pack(u * jnp.tanh(u) + u)

        def ffn2(c0, c1):
            b_scr[:, c0:c1] = jnp.dot(_unpack(h_scr[...]), w2_ref[:, c0:c1],
                                      preferred_element_type=jnp.float32)

        quarter = lax.broadcasted_iota(jnp.int32, (192, 128), 1) // 32
        q32 = lax.broadcasted_iota(jnp.int32, (VR, 128), 1) // 32
        row8 = lax.broadcasted_iota(jnp.int32, (8, 128), 0)

        def partial(j):
            return first and j < 2

        def tile_geom(j, t):
            return (128 * j + 32 * t + 32, 0) if partial(j) else (W + 32, 16 * t)

        def frame_rows(j):
            return 64 * (j + 1) if partial(j) else (W + 128) // 2

        def frame_start(j):
            return 0 if partial(j) else blk * BQ + (128 * j - W)

        def scores(p_ref, col0, j, g, stable):
            for t in range(4):
                nk, fo = tile_geom(j, t)
                kw = k_scr[pl.ds(_al(frame_start(j) // 2 + fo, 8), nk // 2), pl.ds(_al(g * 128, 128), 128)]
                s = jnp.dot(_unpack(kw), _unpack(qm_scr[j, g, t]), preferred_element_type=jnp.float32)
                parts = []
                if not partial(j):
                    parts += [s[0:32] + bias_scr[pl.ds(0, 32), :], s[32:nk - 32]]
                elif nk > 32:
                    parts.append(s[0:nk - 32])
                parts.append(s[nk - 32:nk] + bias_scr[pl.ds(32, 32), :])
                s = jnp.concatenate(parts, axis=0)
                if stable:
                    s = s - jnp.max(s, axis=0, keepdims=True)
                p_ref[pl.ds(z16, nk // 2), pl.ds(col0 + t * 128, 128)] = _pack(jnp.exp2(s))

        def weighted_values(p_ref, col0, j, g):
            nf = frame_rows(j)
            full = []
            for t in range(4):
                nk, fo = tile_geom(j, t)
                parts = [p_ref[pl.ds(z16, nk // 2), pl.ds(col0 + t * 128, 128)]]
                if fo > 0:
                    parts.insert(0, jnp.zeros((fo, 128), jnp.uint32))
                if nf - fo - nk // 2 > 0:
                    parts.append(jnp.zeros((nf - fo - nk // 2, 128), jnp.uint32))
                full.append(jnp.concatenate(parts, axis=0))
            dens, outs = [], []
            for hh in range(4):
                p = full[hh ^ 3]
                for c in (2, 1, 0):
                    p = jnp.where(quarter[0:nf] == c, full[hh ^ c], p)
                vw = vt_scr[4 * g + hh, :, pl.ds(_al(frame_start(j), 128), 2 * nf)]
                out = jnp.dot(vw, _unpack(p), preferred_element_type=jnp.float32)
                r = VR - 1 if hh % 2 == 0 else 0
                den = out[r:r + 1, :]
                on = out * (1.0 / den)
                if hh == 2:
                    on = pltpu.roll(on, 64, 1)
                elif hh != 0:
                    on = jnp.where(q32 % 2 == (0 if hh == 3 else 1),
                                   pltpu.roll(on, 32, 1), pltpu.roll(on, 96, 1))
                dens.append(den)
                outs.append(on)
                if hh % 2 == 1:
                    a, b = outs[hh - 1], outs[hh]
                    pair = jnp.concatenate(
                        [a[0:16], jnp.where(row8 < 4, a[16:24], b[0:8]), b[8:24]], axis=0)
                    ot_scr[pl.ds(_al(80 * g + 20 * (hh - 1), 8), 40), pl.ds(128 * j, 128)] = pair
            return dens

        if first:
            units = [[(0, g), (1, g)] for g in range(NG)]
            units += [[(j, g)] for j in range(2, NJ) for g in range(NG)]
        else:
            units = [[(j, g)] for j in range(NJ) for g in range(NG)]
        pb = (p0, p1)
        dens = []

        def unit_scores(u):
            for idx, (j, g) in enumerate(units[u]):
                scores(pb[u % 2], 512 * idx, j, g, False)

        def unit_values(u):
            for idx, (j, g) in enumerate(units[u]):
                dens.extend(weighted_values(pb[u % 2], 512 * idx, j, g))

        def attention(filler=None):
            unit_scores(0)
            for u in range(len(units)):
                if u + 1 < len(units):
                    unit_scores(u + 1)
                elif filler is not None:
                    filler()
                unit_values(u)

        def finalize():
            o = ot_scr[...].T.astype(jnp.bfloat16)
            a = jnp.dot(o, wo_ref[...], preferred_element_type=jnp.float32)
            b = b_scr[...]
            g = jnp.concatenate([g_scr[...]] * (D // 128), axis=1)
            o_ref[...] = (b + g * (a - b)).astype(o_ref.dtype)

        if first:
            ka = proj(D, D + KC)
            cp_k1.wait()
            kb = proj(D + KC, 2 * D)
            cp_q.wait()
            q = proj(0, D)
            post_k(jnp.concatenate([ka, kb], axis=1))
            cp_v.wait()
            cp_g.wait()
            v = proj(2 * D, 3 * D)
            post_q(q)
            post_v(v)
            gate()
            attention()
            cp_1.wait()
            ffn1()
            cp_2.wait()
            cp_o.wait()
            ffn2(0, D)
        else:
            post_k(proj(D, 2 * D))
            post_q(proj(0, D))
            post_v(proj(2 * D, 3 * D))
            gate()
            ffn1()
            attention(lambda: ffn2(0, 256))
            ffn2(256, D)

        dmin, dmax = dens[0], dens[0]
        for den in dens[1:]:
            dmin = jnp.minimum(dmin, den)
            dmax = jnp.maximum(dmax, den)
        omax = jnp.max(jnp.abs(ot_scr[...]), axis=0, keepdims=True)
        ok = jnp.logical_and(dmin >= DEN_LO, dmax < jnp.inf)
        for j in range(NJ):
            ok = jnp.logical_and(ok, omax[:, 128 * j:128 * (j + 1)] < jnp.inf)
        n_bad = jnp.max(jnp.where(ok, 0, 1))
        finalize()

        @pl.when(n_bad > 0)
        def _():
            for j in range(NJ):
                def group(g, carry, j=j):
                    scores(p0, 0, j, g, True)
                    weighted_values(p0, 0, j, g)
                    return carry
                lax.fori_loop(0, NG, group, 0)
            finalize()

    @pl.when(i == 0)
    def _():
        body(True)

    @pl.when(i > 0)
    def _():
        @pl.when(i + 1 < n_steps)
        def _():
            x_copy(i + 1, 1 - slot).start()
        body(False)


@jax.jit
def pallas_gated_mix__sliding_block__dense_activation_silu__prompt_kernel(
    A_x: jax.Array,
    A_wqkv: jax.Array,
    A_wo: jax.Array,
    B_x: jax.Array,
    B_w1: jax.Array,
    B_w2: jax.Array,
    gate_w: jax.Array,
):
    del B_x
    any_spec = pl.BlockSpec(memory_space=pl.ANY)
    out = pl.pallas_call(
        _kernel,
        grid=(S // BQ,),
        in_specs=[any_spec] * 6,
        out_specs=pl.BlockSpec((BQ, D), lambda i: (i, 0)),
        out_shape=jax.ShapeDtypeStruct((S, D), A_x.dtype),
        scratch_shapes=[
            pltpu.VMEM((2, BQ, D), jnp.bfloat16),
            pltpu.VMEM((D, 3 * D), jnp.bfloat16),
            pltpu.VMEM((D, D), jnp.bfloat16),
            pltpu.VMEM((D, F), jnp.bfloat16),
            pltpu.VMEM((F, D), jnp.bfloat16),
            pltpu.VMEM((D,), jnp.bfloat16),
            pltpu.VMEM((S // 2, NG * 128), jnp.uint32),
            pltpu.VMEM((H, VR, S), jnp.float32),
            pltpu.VMEM((NJ, NG, 4, 64, 128), jnp.uint32),
            pltpu.VMEM((144 + 16, 1024), jnp.uint32),
            pltpu.VMEM((144 + 16, 1024), jnp.uint32),
            pltpu.VMEM((D, BQ), jnp.float32),
            pltpu.VMEM((BQ // 2, F), jnp.uint32),
            pltpu.VMEM((BQ, D), jnp.float32),
            pltpu.VMEM((BQ, 128), jnp.float32),
            pltpu.VMEM((64, 128), jnp.float32),
            pltpu.SemaphoreType.DMA((2,)),
            pltpu.SemaphoreType.DMA((8,)),
        ],
        compiler_params=pltpu.CompilerParams(
            dimension_semantics=("arbitrary",),
            vmem_limit_bytes=100 * 1024 * 1024,
        ),
    )(A_x.reshape(S, D), A_wqkv, A_wo, B_w1, B_w2, gate_w)
    return out.reshape(1, S, D)
```

```python
import numpy as np
import jax
import jax.numpy as jnp
from jax import lax
import jax.experimental.pallas as pl
import jax.experimental.pallas.tpu as pltpu

S = 2048
D = 640
F = 1536
H = 32
DH = 20
W = 256
BQ = 256
NJ = BQ // 128
NG = 8
VR = 24
NEG = -1e30
QSCALE = float(np.log2(np.e)) * (DH ** -0.5)
SLAB_START = (0, 64, 128, 192, 320, 384, 448, 512)
DEN_LO = 2.0 ** -60
KC = 256


def _head_lane0(h):
    st = SLAB_START[h // 4]
    col = DH * h
    return col - st if st % 128 == 0 else (col - st + 64) % 128


def _slab(v, g, lane_hi):
    st = SLAB_START[g]
    if st % 128 == 0:
        return v[:, st:st + 128]
    m = st // 128
    return jnp.where(lane_hi, v[:, 128 * m:128 * (m + 1)], v[:, 128 * (m + 1):128 * (m + 2)])


def _pack(x):
    return pltpu.bitcast(x.astype(jnp.bfloat16), jnp.uint32)


def _unpack(x):
    return pltpu.bitcast(x, jnp.bfloat16)


def _dot5(x, w_ref, c0):
    lo = jnp.dot(x, w_ref[:, c0:c0 + 512], preferred_element_type=jnp.float32)
    hi = [jnp.dot(x[64 * c:64 * (c + 1)], w_ref[:, c0 + 512:c0 + D], preferred_element_type=jnp.float32)
          for c in range(BQ // 64)]
    return jnp.concatenate([lo, jnp.concatenate(hi, axis=0)], axis=1)


def _al(x, n):
    return x if isinstance(x, int) else pl.multiple_of(x, n)


def _kernel(x_hbm, wqkv_hbm, wo_hbm, w1_hbm, w2_hbm, gw_hbm, o_ref,
            x_buf, wqkv_ref, wo_ref, w1_ref, w2_ref, gw_ref,
            k_scr, vt_scr, qm_scr, p0, p1, ot_scr, h_scr, b_scr, g_scr, bias_scr,
            xsem, wsem):
    i = pl.program_id(0)
    n_steps = S // BQ
    z16 = pl.multiple_of(jnp.minimum(i, 0) * 16, 16)
    slot = i % 2

    def x_copy(blk, sl):
        return pltpu.make_async_copy(x_hbm.at[pl.ds(_al(blk * BQ, BQ), BQ), :], x_buf.at[sl], xsem.at[sl])

    def w_copy(src, dst, sem):
        return pltpu.make_async_copy(src, dst, wsem.at[sem])

    cp_k0 = w_copy(wqkv_hbm.at[:, pl.ds(D, KC)], wqkv_ref.at[:, pl.ds(D, KC)], 0)
    cp_k1 = w_copy(wqkv_hbm.at[:, pl.ds(D + KC, D - KC)], wqkv_ref.at[:, pl.ds(D + KC, D - KC)], 1)
    cp_q = w_copy(wqkv_hbm.at[:, pl.ds(0, D)], wqkv_ref.at[:, pl.ds(0, D)], 2)
    cp_v = w_copy(wqkv_hbm.at[:, pl.ds(2 * D, D)], wqkv_ref.at[:, pl.ds(2 * D, D)], 3)
    cp_g = w_copy(gw_hbm, gw_ref, 4)
    cp_1 = w_copy(w1_hbm, w1_ref, 5)
    cp_2 = w_copy(w2_hbm, w2_ref, 6)
    cp_o = w_copy(wo_hbm, wo_ref, 7)

    def body(first):
        blk = 0 if first else i
        if first:
            x_copy(0, 0).start()
            cp_k0.start()
            for cp in (cp_k1, cp_q, cp_v, cp_g, cp_1, cp_2, cp_o, x_copy(1, 1)):
                cp.start(priority=1)
            ri = lax.broadcasted_iota(jnp.int32, (32, 128), 0)
            li = lax.broadcasted_iota(jnp.int32, (32, 128), 1) % 32
            bias_scr[pl.ds(0, 32), :] = jnp.where(ri > li, 0.0, NEG)
            bias_scr[pl.ds(32, 32), :] = jnp.where(ri <= li, 0.0, NEG)
            x_copy(0, 0).wait()
            cp_k0.wait()
            x = x_buf[0]
        else:
            x_copy(i, slot).wait()
            x = x_buf[slot]

        lane_hi = lax.broadcasted_iota(jnp.int32, (BQ, 128), 1) >= 64
        lane1 = lax.broadcasted_iota(jnp.int32, (1, 128), 1)

        def proj(c0, c1):
            if c1 - c0 == D:
                return _dot5(x, wqkv_ref, c0)
            return jnp.dot(x, wqkv_ref[:, c0:c1], preferred_element_type=jnp.float32)

        def post_k(k):
            kext = jnp.concatenate([_slab(k, g, lane_hi) for g in range(NG)], axis=1)
            k_scr[pl.ds(_al(blk * (BQ // 2), BQ // 2), BQ // 2), :] = _pack(kext)

        def post_q(q):
            for g in range(NG):
                qg = _slab(q, g, lane_hi)
                lms = [jnp.where(((lane1 - _head_lane0(4 * g + hh)) & 127) < DH, QSCALE, 0.0)
                       for hh in range(4)]
                for j in range(NJ):
                    for t in range(4):
                        rows = qg[128 * j + 32 * t:128 * j + 32 * t + 32]
                        tile = jnp.concatenate(
                            [(rows * lms[c ^ t]).astype(jnp.bfloat16) for c in range(4)], axis=0)
                        qm_scr[j, g, t] = pltpu.bitcast(tile.T, jnp.uint32)

        def post_v(v):
            vt = v.T.astype(jnp.bfloat16).astype(jnp.float32)
            rowv = lax.broadcasted_iota(jnp.int32, (VR, BQ), 0)
            for h in range(H):
                w0 = 8 * ((DH * h) // 8)
                ones_row = VR - 1 if h % 2 == 0 else 0
                vt_scr[h, :, pl.ds(_al(blk * BQ, BQ), BQ)] = jnp.where(
                    rowv == ones_row, 1.0, vt[w0:w0 + VR, :])

        def gate():
            gw = gw_ref[...].astype(jnp.float32).reshape(1, D)
            gl = jnp.sum(x.astype(jnp.float32) * gw, axis=-1, keepdims=True)
            g_scr[...] = jnp.broadcast_to(0.5 * jnp.tanh(0.5 * gl) + 0.5, (BQ, 128))

        def ffn1():
            u = 0.5 * jnp.dot(x, w1_ref[...], preferred_element_type=jnp.float32)
            h_scr[...] = _pack(u * jnp.tanh(u) + u)

        def ffn2(c0, c1):
            b_scr[:, c0:c1] = jnp.dot(_unpack(h_scr[...]), w2_ref[:, c0:c1],
                                      preferred_element_type=jnp.float32)

        quarter = lax.broadcasted_iota(jnp.int32, (192, 128), 1) // 32
        q32 = lax.broadcasted_iota(jnp.int32, (VR, 128), 1) // 32
        row8 = lax.broadcasted_iota(jnp.int32, (8, 128), 0)

        def partial(j):
            return first and j < 2

        def tile_geom(j, t):
            return (128 * j + 32 * t + 32, 0) if partial(j) else (W + 32, 16 * t)

        def frame_rows(j):
            return 64 * (j + 1) if partial(j) else (W + 128) // 2

        def frame_start(j):
            return 0 if partial(j) else blk * BQ + (128 * j - W)

        def scores(p_ref, col0, j, g, stable):
            for t in range(4):
                nk, fo = tile_geom(j, t)
                kw = k_scr[pl.ds(_al(frame_start(j) // 2 + fo, 8), nk // 2), pl.ds(_al(g * 128, 128), 128)]
                s = jnp.dot(_unpack(kw), _unpack(qm_scr[j, g, t]), preferred_element_type=jnp.float32)
                parts = []
                if not partial(j):
                    parts += [s[0:32] + bias_scr[pl.ds(0, 32), :], s[32:nk - 32]]
                elif nk > 32:
                    parts.append(s[0:nk - 32])
                parts.append(s[nk - 32:nk] + bias_scr[pl.ds(32, 32), :])
                s = jnp.concatenate(parts, axis=0)
                if stable:
                    s = s - jnp.max(s, axis=0, keepdims=True)
                p_ref[pl.ds(z16, nk // 2), pl.ds(col0 + t * 128, 128)] = _pack(jnp.exp2(s))

        def weighted_values(p_ref, col0, j, g):
            nf = frame_rows(j)
            full = []
            for t in range(4):
                nk, fo = tile_geom(j, t)
                parts = [p_ref[pl.ds(z16, nk // 2), pl.ds(col0 + t * 128, 128)]]
                if fo > 0:
                    parts.insert(0, jnp.zeros((fo, 128), jnp.uint32))
                if nf - fo - nk // 2 > 0:
                    parts.append(jnp.zeros((nf - fo - nk // 2, 128), jnp.uint32))
                full.append(jnp.concatenate(parts, axis=0))
            dens, outs = [], []
            for hh in range(4):
                p = full[hh ^ 3]
                for c in (2, 1, 0):
                    p = jnp.where(quarter[0:nf] == c, full[hh ^ c], p)
                vw = vt_scr[4 * g + hh, :, pl.ds(_al(frame_start(j), 128), 2 * nf)]
                out = jnp.dot(vw, _unpack(p), preferred_element_type=jnp.float32)
                r = VR - 1 if hh % 2 == 0 else 0
                den = out[r:r + 1, :]
                on = out * (1.0 / den)
                if hh == 2:
                    on = pltpu.roll(on, 64, 1)
                elif hh != 0:
                    on = jnp.where(q32 % 2 == (0 if hh == 3 else 1),
                                   pltpu.roll(on, 32, 1), pltpu.roll(on, 96, 1))
                dens.append(den)
                outs.append(on)
                if hh % 2 == 1:
                    a, b = outs[hh - 1], outs[hh]
                    pair = jnp.concatenate(
                        [a[0:16], jnp.where(row8 < 4, a[16:24], b[0:8]), b[8:24]], axis=0)
                    ot_scr[pl.ds(_al(80 * g + 20 * (hh - 1), 8), 40), pl.ds(128 * j, 128)] = pair
            return dens

        if first:
            units = [[(0, g), (1, g)] for g in range(NG)]
            units += [[(j, g)] for j in range(2, NJ) for g in range(NG)]
        else:
            units = [[(j, g)] for j in range(NJ) for g in range(NG)]
        pb = (p0, p1)
        dens = []

        def unit_scores(u):
            for idx, (j, g) in enumerate(units[u]):
                scores(pb[u % 2], 512 * idx, j, g, False)

        def unit_values(u):
            for idx, (j, g) in enumerate(units[u]):
                dens.extend(weighted_values(pb[u % 2], 512 * idx, j, g))

        def attention(filler=None, hook=None):
            unit_scores(0)
            for u in range(len(units)):
                if hook is not None:
                    hook(u)
                if u + 1 < len(units):
                    unit_scores(u + 1)
                elif filler is not None:
                    filler()
                unit_values(u)

        def finalize():
            o = ot_scr[...].T.astype(jnp.bfloat16)
            a = _dot5(o, wo_ref, 0)
            b = b_scr[...]
            g = jnp.concatenate([g_scr[...]] * (D // 128), axis=1)
            o_ref[...] = (b + g * (a - b)).astype(o_ref.dtype)

        if first:
            ka = proj(D, D + KC)
            cp_k1.wait()
            kb = proj(D + KC, 2 * D)
            cp_q.wait()
            q = proj(0, D)
            cp_v.wait()
            cp_g.wait()
            v = proj(2 * D, 3 * D)
            post_k(jnp.concatenate([ka, kb], axis=1))
            post_q(q)
            post_v(v)
            gate()
            attention(ffn1, lambda u: cp_1.wait() if u == len(units) - 1 else None)
            cp_2.wait()
            cp_o.wait()
            ffn2(0, D)
        else:
            post_k(proj(D, 2 * D))
            post_q(proj(0, D))
            post_v(proj(2 * D, 3 * D))
            gate()
            ffn1()
            attention(lambda: ffn2(0, 256))
            ffn2(256, D)

        dmin, dmax = dens[0], dens[0]
        for den in dens[1:]:
            dmin = jnp.minimum(dmin, den)
            dmax = jnp.maximum(dmax, den)
        omax = jnp.max(jnp.abs(ot_scr[...]), axis=0, keepdims=True)
        ok = jnp.logical_and(dmin >= DEN_LO, dmax < jnp.inf)
        for j in range(NJ):
            ok = jnp.logical_and(ok, omax[:, 128 * j:128 * (j + 1)] < jnp.inf)
        n_bad = jnp.max(jnp.where(ok, 0, 1))
        finalize()

        @pl.when(n_bad > 0)
        def _():
            for j in range(NJ):
                def group(g, carry, j=j):
                    scores(p0, 0, j, g, True)
                    weighted_values(p0, 0, j, g)
                    return carry
                lax.fori_loop(0, NG, group, 0)
            finalize()

    @pl.when(i == 0)
    def _():
        body(True)

    @pl.when(i > 0)
    def _():
        @pl.when(i + 1 < n_steps)
        def _():
            x_copy(i + 1, 1 - slot).start()
        body(False)


@jax.jit
def pallas_gated_mix__sliding_block__dense_activation_silu__prompt_kernel(
    A_x: jax.Array,
    A_wqkv: jax.Array,
    A_wo: jax.Array,
    B_x: jax.Array,
    B_w1: jax.Array,
    B_w2: jax.Array,
    gate_w: jax.Array,
):
    del B_x
    any_spec = pl.BlockSpec(memory_space=pl.ANY)
    out = pl.pallas_call(
        _kernel,
        grid=(S // BQ,),
        in_specs=[any_spec] * 6,
        out_specs=pl.BlockSpec((BQ, D), lambda i: (i, 0)),
        out_shape=jax.ShapeDtypeStruct((S, D), A_x.dtype),
        scratch_shapes=[
            pltpu.VMEM((2, BQ, D), jnp.bfloat16),
            pltpu.VMEM((D, 3 * D), jnp.bfloat16),
            pltpu.VMEM((D, D), jnp.bfloat16),
            pltpu.VMEM((D, F), jnp.bfloat16),
            pltpu.VMEM((F, D), jnp.bfloat16),
            pltpu.VMEM((D,), jnp.bfloat16),
            pltpu.VMEM((S // 2, NG * 128), jnp.uint32),
            pltpu.VMEM((H, VR, S), jnp.float32),
            pltpu.VMEM((NJ, NG, 4, 64, 128), jnp.uint32),
            pltpu.VMEM((144 + 16, 1024), jnp.uint32),
            pltpu.VMEM((144 + 16, 1024), jnp.uint32),
            pltpu.VMEM((D, BQ), jnp.float32),
            pltpu.VMEM((BQ // 2, F), jnp.uint32),
            pltpu.VMEM((BQ, D), jnp.float32),
            pltpu.VMEM((BQ, 128), jnp.float32),
            pltpu.VMEM((64, 128), jnp.float32),
            pltpu.SemaphoreType.DMA((2,)),
            pltpu.SemaphoreType.DMA((8,)),
        ],
        compiler_params=pltpu.CompilerParams(
            dimension_semantics=("arbitrary",),
            vmem_limit_bytes=100 * 1024 * 1024,
        ),
    )(A_x.reshape(S, D), A_wqkv, A_wo, B_w1, B_w2, gate_w)
    return out.reshape(1, S, D)
```

```python
import numpy as np
import jax
import jax.numpy as jnp
from jax import lax
import jax.experimental.pallas as pl
import jax.experimental.pallas.tpu as pltpu

S = 2048
D = 640
F = 1536
H = 32
DH = 20
W = 256
BQ = 256
NJ = BQ // 128
NG = 8
VR = 24
NEG = -1e30
QSCALE = float(np.log2(np.e)) * (DH ** -0.5)
SLAB_START = (0, 64, 128, 192, 320, 384, 448, 512)
DEN_LO_BITS = int(np.float32(2.0 ** -60).view(np.int32))
INF_BITS = 0x7F800000
KC = 256


def _head_lane0(h):
    st = SLAB_START[h // 4]
    col = DH * h
    return col - st if st % 128 == 0 else (col - st + 64) % 128


def _slab(v, g, lane_hi):
    st = SLAB_START[g]
    if st % 128 == 0:
        return v[:, st:st + 128]
    m = st // 128
    return jnp.where(lane_hi, v[:, 128 * m:128 * (m + 1)], v[:, 128 * (m + 1):128 * (m + 2)])


def _pack(x):
    return pltpu.bitcast(x.astype(jnp.bfloat16), jnp.uint32)


def _unpack(x):
    return pltpu.bitcast(x, jnp.bfloat16)


def _dot5(x, w_ref, c0):
    lo = jnp.dot(x, w_ref[:, c0:c0 + 512], preferred_element_type=jnp.float32)
    hi = [jnp.dot(x[64 * c:64 * (c + 1)], w_ref[:, c0 + 512:c0 + D], preferred_element_type=jnp.float32)
          for c in range(BQ // 64)]
    return jnp.concatenate([lo, jnp.concatenate(hi, axis=0)], axis=1)


def _al(x, n):
    return x if isinstance(x, int) else pl.multiple_of(x, n)


def _kernel(x_hbm, wqkv_hbm, wo_hbm, w1_hbm, w2_hbm, gw_hbm, o_ref,
            x_buf, wqkv_ref, wo_ref, w1_ref, w2_ref, gw_ref,
            k_scr, vt_scr, qm_scr, p0, p1, ot_scr, h_scr, b_scr, g_scr, bias_scr,
            xsem, wsem):
    i = pl.program_id(0)
    n_steps = S // BQ
    z16 = pl.multiple_of(jnp.minimum(i, 0) * 16, 16)
    slot = i % 2

    def x_copy(blk, sl):
        return pltpu.make_async_copy(x_hbm.at[pl.ds(_al(blk * BQ, BQ), BQ), :], x_buf.at[sl], xsem.at[sl])

    def w_copy(src, dst, sem):
        return pltpu.make_async_copy(src, dst, wsem.at[sem])

    cp_k0 = w_copy(wqkv_hbm.at[:, pl.ds(D, KC)], wqkv_ref.at[:, pl.ds(D, KC)], 0)
    cp_k1 = w_copy(wqkv_hbm.at[:, pl.ds(D + KC, D - KC)], wqkv_ref.at[:, pl.ds(D + KC, D - KC)], 1)
    cp_q = w_copy(wqkv_hbm.at[:, pl.ds(0, D)], wqkv_ref.at[:, pl.ds(0, D)], 2)
    cp_v = w_copy(wqkv_hbm.at[:, pl.ds(2 * D, D)], wqkv_ref.at[:, pl.ds(2 * D, D)], 3)
    cp_g = w_copy(gw_hbm, gw_ref, 4)
    cp_1 = w_copy(w1_hbm, w1_ref, 5)
    cp_2 = w_copy(w2_hbm, w2_ref, 6)
    cp_o = w_copy(wo_hbm, wo_ref, 7)

    def body(first):
        blk = 0 if first else i
        if first:
            x_copy(0, 0).start()
            cp_k0.start()
            for cp in (cp_k1, cp_q, cp_v, cp_g, cp_1, cp_2, cp_o, x_copy(1, 1)):
                cp.start(priority=1)
            ri = lax.broadcasted_iota(jnp.int32, (32, 128), 0)
            li = lax.broadcasted_iota(jnp.int32, (32, 128), 1) % 32
            bias_scr[pl.ds(0, 32), :] = jnp.where(ri > li, 0.0, NEG)
            bias_scr[pl.ds(32, 32), :] = jnp.where(ri <= li, 0.0, NEG)
            x_copy(0, 0).wait()
            cp_k0.wait()
            x = x_buf[0]
        else:
            x_copy(i, slot).wait()
            x = x_buf[slot]

        lane_hi = lax.broadcasted_iota(jnp.int32, (BQ, 128), 1) >= 64
        lane1 = lax.broadcasted_iota(jnp.int32, (1, 128), 1)

        def proj(c0, c1):
            if c1 - c0 == D:
                return _dot5(x, wqkv_ref, c0)
            return jnp.dot(x, wqkv_ref[:, c0:c1], preferred_element_type=jnp.float32)

        def post_k(k):
            kext = jnp.concatenate([_slab(k, g, lane_hi) for g in range(NG)], axis=1)
            k_scr[pl.ds(_al(blk * (BQ // 2), BQ // 2), BQ // 2), :] = _pack(kext)

        def post_q(q):
            for g in range(NG):
                qg = _slab(q, g, lane_hi)
                lms = [jnp.where(((lane1 - _head_lane0(4 * g + hh)) & 127) < DH, QSCALE, 0.0)
                       for hh in range(4)]
                for j in range(NJ):
                    for t in range(4):
                        rows = qg[128 * j + 32 * t:128 * j + 32 * t + 32]
                        tile = jnp.concatenate(
                            [(rows * lms[c ^ t]).astype(jnp.bfloat16) for c in range(4)], axis=0)
                        qm_scr[j, g, t] = pltpu.bitcast(tile.T, jnp.uint32)

        def post_v(v):
            vt = v.T.astype(jnp.bfloat16).astype(jnp.float32)
            rowv = lax.broadcasted_iota(jnp.int32, (VR, BQ), 0)
            for h in range(H):
                w0 = 8 * ((DH * h) // 8)
                ones_row = VR - 1 if h % 2 == 0 else 0
                vt_scr[h, :, pl.ds(_al(blk * BQ, BQ), BQ)] = jnp.where(
                    rowv == ones_row, 1.0, vt[w0:w0 + VR, :])

        def gate():
            gw = gw_ref[...].astype(jnp.float32).reshape(1, D)
            gl = jnp.sum(x.astype(jnp.float32) * gw, axis=-1, keepdims=True)
            g_scr[...] = jnp.broadcast_to(0.5 * jnp.tanh(0.5 * gl) + 0.5, (BQ, 128))

        def ffn1():
            u = 0.5 * jnp.dot(x, w1_ref[...], preferred_element_type=jnp.float32)
            h_scr[...] = _pack(u * jnp.tanh(u) + u)

        def ffn2(c0, c1):
            b_scr[:, c0:c1] = jnp.dot(_unpack(h_scr[...]), w2_ref[:, c0:c1],
                                      preferred_element_type=jnp.float32)

        quarter = lax.broadcasted_iota(jnp.int32, (192, 128), 1) // 32
        q32 = lax.broadcasted_iota(jnp.int32, (VR, 128), 1) // 32
        row8 = lax.broadcasted_iota(jnp.int32, (8, 128), 0)

        def partial(j):
            return first and j < 2

        def tile_geom(j, t):
            return (128 * j + 32 * t + 32, 0) if partial(j) else (W + 32, 16 * t)

        def frame_rows(j):
            return 64 * (j + 1) if partial(j) else (W + 128) // 2

        def frame_start(j):
            return 0 if partial(j) else blk * BQ + (128 * j - W)

        def scores(p_ref, col0, j, g, stable):
            for t in range(4):
                nk, fo = tile_geom(j, t)
                kw = k_scr[pl.ds(_al(frame_start(j) // 2 + fo, 8), nk // 2), pl.ds(_al(g * 128, 128), 128)]
                s = jnp.dot(_unpack(kw), _unpack(qm_scr[j, g, t]), preferred_element_type=jnp.float32)
                parts = []
                if not partial(j):
                    parts += [s[0:32] + bias_scr[pl.ds(0, 32), :], s[32:nk - 32]]
                elif nk > 32:
                    parts.append(s[0:nk - 32])
                parts.append(s[nk - 32:nk] + bias_scr[pl.ds(32, 32), :])
                s = jnp.concatenate(parts, axis=0)
                if stable:
                    s = s - jnp.max(s, axis=0, keepdims=True)
                p_ref[pl.ds(z16, nk // 2), pl.ds(col0 + t * 128, 128)] = _pack(jnp.exp2(s))

        def weighted_values(p_ref, col0, j, g):
            nf = frame_rows(j)
            full = []
            for t in range(4):
                nk, fo = tile_geom(j, t)
                parts = [p_ref[pl.ds(z16, nk // 2), pl.ds(col0 + t * 128, 128)]]
                if fo > 0:
                    parts.insert(0, jnp.zeros((fo, 128), jnp.uint32))
                if nf - fo - nk // 2 > 0:
                    parts.append(jnp.zeros((nf - fo - nk // 2, 128), jnp.uint32))
                full.append(jnp.concatenate(parts, axis=0))
            dens, outs = [], []
            for hh in range(4):
                p = full[hh ^ 3]
                for c in (2, 1, 0):
                    p = jnp.where(quarter[0:nf] == c, full[hh ^ c], p)
                vw = vt_scr[4 * g + hh, :, pl.ds(_al(frame_start(j), 128), 2 * nf)]
                out = jnp.dot(vw, _unpack(p), preferred_element_type=jnp.float32)
                r = VR - 1 if hh % 2 == 0 else 0
                den = out[r:r + 1, :]
                on = out * (1.0 / den)
                if hh == 2:
                    on = pltpu.roll(on, 64, 1)
                elif hh != 0:
                    on = jnp.where(q32 % 2 == (0 if hh == 3 else 1),
                                   pltpu.roll(on, 32, 1), pltpu.roll(on, 96, 1))
                dens.append(den)
                outs.append(on)
                if hh % 2 == 1:
                    a, b = outs[hh - 1], outs[hh]
                    pair = jnp.concatenate(
                        [a[0:16], jnp.where(row8 < 4, a[16:24], b[0:8]), b[8:24]], axis=0)
                    ot_scr[pl.ds(_al(80 * g + 20 * (hh - 1), 8), 40), pl.ds(128 * j, 128)] = pair
            return dens

        if first:
            units = [[(0, g), (1, g)] for g in range(NG)]
            units += [[(j, g)] for j in range(2, NJ) for g in range(NG)]
        else:
            units = [[(j, g)] for j in range(NJ) for g in range(NG)]
        pb = (p0, p1)
        dens = []

        def unit_scores(u):
            for idx, (j, g) in enumerate(units[u]):
                scores(pb[u % 2], 512 * idx, j, g, False)

        def unit_values(u):
            for idx, (j, g) in enumerate(units[u]):
                dens.extend(weighted_values(pb[u % 2], 512 * idx, j, g))

        def attention(filler=None, hook=None):
            unit_scores(0)
            for u in range(len(units)):
                if hook is not None:
                    hook(u)
                if u + 1 < len(units):
                    unit_scores(u + 1)
                elif filler is not None:
                    filler()
                unit_values(u)

        def finalize():
            o = ot_scr[...].T.astype(jnp.bfloat16)
            a = _dot5(o, wo_ref, 0)
            b = b_scr[...]
            g = jnp.concatenate([g_scr[...]] * (D // 128), axis=1)
            o_ref[...] = (b + g * (a - b)).astype(o_ref.dtype)

        if first:
            ka = proj(D, D + KC)
            cp_k1.wait()
            kb = proj(D + KC, 2 * D)
            cp_q.wait()
            q = proj(0, D)
            cp_v.wait()
            cp_g.wait()
            v = proj(2 * D, 3 * D)
            post_k(jnp.concatenate([ka, kb], axis=1))
            post_q(q)
            post_v(v)
            gate()
            attention(ffn1, lambda u: cp_1.wait() if u == len(units) - 1 else None)
            cp_2.wait()
            cp_o.wait()
            ffn2(0, D)
        else:
            post_k(proj(D, 2 * D))
            post_q(proj(0, D))
            post_v(proj(2 * D, 3 * D))
            gate()
            ffn1()
            attention(lambda: ffn2(0, 256))
            ffn2(256, D)

        dbits = [lax.bitcast_convert_type(den, jnp.int32) for den in dens]
        dmin, dmax = dbits[0], dbits[0]
        for d in dbits[1:]:
            dmin = jnp.minimum(dmin, d)
            dmax = jnp.maximum(dmax, d)
        obits = lax.bitcast_convert_type(ot_scr[...], jnp.int32) & 0x7FFFFFFF
        omax = jnp.max(obits, axis=0, keepdims=True)
        ok = jnp.logical_and(dmin >= DEN_LO_BITS, dmax < INF_BITS)
        for j in range(NJ):
            ok = jnp.logical_and(ok, omax[:, 128 * j:128 * (j + 1)] < INF_BITS)
        n_bad = jnp.max(jnp.where(ok, 0, 1))
        finalize()

        @pl.when(n_bad > 0)
        def _():
            for j in range(NJ):
                def group(g, carry, j=j):
                    scores(p0, 0, j, g, True)
                    weighted_values(p0, 0, j, g)
                    return carry
                lax.fori_loop(0, NG, group, 0)
            finalize()

    @pl.when(i == 0)
    def _():
        body(True)

    @pl.when(i > 0)
    def _():
        @pl.when(i + 1 < n_steps)
        def _():
            x_copy(i + 1, 1 - slot).start()
        body(False)


@jax.jit
def pallas_gated_mix__sliding_block__dense_activation_silu__prompt_kernel(
    A_x: jax.Array,
    A_wqkv: jax.Array,
    A_wo: jax.Array,
    B_x: jax.Array,
    B_w1: jax.Array,
    B_w2: jax.Array,
    gate_w: jax.Array,
):
    del B_x
    any_spec = pl.BlockSpec(memory_space=pl.ANY)
    out = pl.pallas_call(
        _kernel,
        grid=(S // BQ,),
        in_specs=[any_spec] * 6,
        out_specs=pl.BlockSpec((BQ, D), lambda i: (i, 0)),
        out_shape=jax.ShapeDtypeStruct((S, D), A_x.dtype),
        scratch_shapes=[
            pltpu.VMEM((2, BQ, D), jnp.bfloat16),
            pltpu.VMEM((D, 3 * D), jnp.bfloat16),
            pltpu.VMEM((D, D), jnp.bfloat16),
            pltpu.VMEM((D, F), jnp.bfloat16),
            pltpu.VMEM((F, D), jnp.bfloat16),
            pltpu.VMEM((D,), jnp.bfloat16),
            pltpu.VMEM((S // 2, NG * 128), jnp.uint32),
            pltpu.VMEM((H, VR, S), jnp.float32),
            pltpu.VMEM((NJ, NG, 4, 64, 128), jnp.uint32),
            pltpu.VMEM((144 + 16, 1024), jnp.uint32),
            pltpu.VMEM((144 + 16, 1024), jnp.uint32),
            pltpu.VMEM((D, BQ), jnp.float32),
            pltpu.VMEM((BQ // 2, F), jnp.uint32),
            pltpu.VMEM((BQ, D), jnp.float32),
            pltpu.VMEM((BQ, 128), jnp.float32),
            pltpu.VMEM((64, 128), jnp.float32),
            pltpu.SemaphoreType.DMA((2,)),
            pltpu.SemaphoreType.DMA((8,)),
        ],
        compiler_params=pltpu.CompilerParams(
            dimension_semantics=("arbitrary",),
            vmem_limit_bytes=64 * 1024 * 1024,
        ),
    )(A_x.reshape(S, D), A_wqkv, A_wo, B_w1, B_w2, gate_w)
    return out.reshape(1, S, D)
```
